```python
import jax
import jax.numpy as jnp

def _softmax(x, axis=-1):
    return jax.nn.softmax(x, axis=axis)
def _gelu(x):
    return jax.nn.gelu(x, approximate=True)
def _silu(x):
    return jax.nn.silu(x)
def _sigmoid(x):
    return jax.nn.sigmoid(x)
def _layernorm(x, axis=-1, eps=1e-5):
    m = jnp.mean(x, axis=axis, keepdims=True)
    v = jnp.var(x, axis=axis, keepdims=True)
    return (x - m) / jnp.sqrt(v + eps)
def _scatter_add(tgt, idx, src, axis=0):
    return tgt.at[idx].add(src)
def _segment_sum(src, seg, n):
    return jax.ops.segment_sum(src, seg, n)
class _Rng:
    def __init__(self, key):
        self._k = key
    def _next(self):
        self._k, sub = jax.random.split(self._k)
        return sub
    def normal(self, shape):
        return jax.random.normal(self._next(), shape, dtype=jnp.bfloat16)
    def randint(self, lo, hi, shape):
        return jax.random.randint(self._next(), shape, lo, hi, dtype=jnp.int32)
    def uniform(self, shape, lo=0.0, hi=1.0):
        return jax.random.uniform(self._next(), shape, jnp.bfloat16, lo, hi)
    def permutation(self, n):
        return jax.random.permutation(self._next(), n)


kernel_name = 'standalone__modern_conv_block_convnext__vision'

def setup_inputs():
    _rng = _Rng(jax.random.key(int.from_bytes(__import__("os").urandom(4), "little")))
    _w = (lambda a: (lambda t: t.astype(jnp.bfloat16) if jnp.issubdtype(t.dtype, jnp.floating) else t)(jnp.asarray(a)))
    H = W = 512
    C = 96
    K = 3
    return {
        "x": _w((lambda *s: _rng.normal(s) * 0.05)(1, H, W, C)),
        "dw": _w((lambda *s: _rng.normal(s) * 0.05)(K, K, C)),
        "w1": _w((lambda *s: _rng.normal(s) * 0.05)(C, 4 * C)),
        "b1": _w((lambda *s: _rng.normal(s) * 0.05)(4 * C)),
        "w2": _w((lambda *s: _rng.normal(s) * 0.05)(4 * C, C)),
        "b2": _w((lambda *s: _rng.normal(s) * 0.05)(C)),
        "gamma": _w((lambda *s: _rng.normal(s) * 0.05)(C)),
    }

def reference(x, dw, w1, b1, w2, b2, gamma):
    B, H, W, C = x.shape
    K = dw.shape[0]
    pad = K // 2
    xp = jnp.pad(x, ((0,0),(pad,pad),(pad,pad),(0,0)))
    out = jnp.zeros_like(x)
    for i in range(K):
        for j in range(K):
            out = out + xp[:, i:i+H, j:j+W, :] * dw[i, j][None, None, None, :]
    h = _layernorm(out, axis=-1)
    h = jnp.einsum('bhwc,ce->bhwe', h, w1) + b1
    h = _gelu(h)
    h = jnp.einsum('bhwe,ec->bhwc', h, w2) + b2
    return x + gamma[None, None, None, :] * h
```

```python
import functools, contextlib
import jax, jax.numpy as jnp, numpy as np
from jax import lax
from jax.experimental import pallas as pl
from jax.experimental.pallas import tpu as pltpu

A_ = float(np.sqrt(2.0/np.pi)); B_ = A_*0.044715
S_ = B_ ** (1.0/3.0)
AP = A_/S_
EPS = 1e-5
H = W = 512; C = 96; E = 384; NQ = 4
f32 = jnp.float32; bf16 = jnp.bfloat16; u32 = jnp.uint32

def seq(a, n=12, off=0): return ' '.join(f"{a}{g}" for g in range(off, off+n))

def build(dead=None, events=None):
    ev = [(16*c, 1, f"w{c}") for c in range(24)] + [(384+16*i, 1, f"x{i}") for i in range(18)]
    ev = [(t, 0, op) for t, op in events] + ev
    ev.sort(key=lambda e: (e[0], e[1]))
    return ' '.join(e[2] for e in ev)

def make(prog, first=None, last=None, R=4, form='R', accmem=True, hold=False, flags=None, tq=3):
    NCH = H // R
    NS = 4
    L = 3
    assert R % NS == 0 and R >= L
    parse = lambda p: [(t[0], int(t[1:]) if len(t) > 1 else 0) for t in p.split()]
    iP0, iP1, iXC, iCV, iS1, iW, iTOK, iXN, iWT = 0, 1, 2, 6, 7, 8, 11, 12, 13
    def kern(x_hbm, dw_ref, w1_ref, b1_ref, w2t_ref, b2_ref, g_ref, o_hbm,
             xin, xpre, obuf, vs, wts, accA, accB, b2b, zs, isem, osem, psem):
        def in_copy(j, slot):
            return pltpu.make_async_copy(x_hbm.at[pl.ds(j*R+L, R)], xin.at[slot], isem.at[slot])
        def in_copy_last(slot):
            return pltpu.make_async_copy(x_hbm.at[pl.ds(H-R+L, R-L)], xin.at[slot, pl.ds(0, R-L)], isem.at[slot])
        def out_copy(j, slot):
            return pltpu.make_async_copy(obuf.at[slot], o_hbm.at[pl.ds(j*R, R)], osem.at[slot])
        pre = pltpu.make_async_copy(x_hbm.at[pl.ds(0, L)], xpre, psem)
        pre.start()
        in_copy(0, 0).start()
        zs[0] = 0; zs[1] = 0; zs[2] = 0

        def bcast(row):
            r = jnp.concatenate([row, jnp.zeros((1, 32), f32)], axis=1)
            return jnp.broadcast_to(r, (128, 128)).T[:C]
        dw = dw_ref[...].astype(f32)
        for t in range(9):
            vs[iW + t // 4, :, 128*(t % 4):128*(t % 4)+128] = bcast(dw[t:t+1])
        gb = bcast(g_ref[...].astype(f32))
        b2b[...] = gb * bcast(b2_ref[...].astype(f32))
        w1 = w1_ref[...].astype(f32)
        b1 = b1_ref[...].astype(f32) * S_
        hi = b1.astype(bf16).astype(f32)
        w1e = jnp.concatenate([w1, hi, b1 - hi, jnp.zeros((30, E), f32)], axis=0).T
        def wslot(i): return (slice(8*(i//4), 8*(i//4)+8), slice(128*(i%4), 128*(i%4)+128))
        for k in range(3):
            for c in range(8):
                wts[(0,) + wslot(8*k+c)] = pltpu.bitcast(w1e[128*k+16*(7-c):128*k+16*(8-c)].astype(bf16), f32)
                vs[(iWT,) + wslot(8*k+c)] = pltpu.bitcast(w1e[128*k+16*(7-c):128*k+16*(8-c)].astype(bf16), f32)
        w2 = (w2t_ref[...].astype(f32) * (jnp.concatenate([gb]*3, axis=1) * (0.5/S_)))
        for k in range(3):
            for g in range(6):
                wts[(0,) + wslot(24+6*k+g)] = pltpu.bitcast(w2[16*g:16*g+16, 128*k:128*k+128].astype(bf16), f32)
                vs[(iWT,) + wslot(24+6*k+g)] = pltpu.bitcast(w2[16*g:16*g+16, 128*k:128*k+128].astype(bf16), f32)
        for i in [iP0, iP1] + [iXC+s for s in range(NS)] + [iTOK]:
            vs[i] = jnp.zeros((C, W), f32)

        first_ = lax.broadcasted_iota(jnp.int32, (8, 128), 1) == 0
        last_ = lax.broadcasted_iota(jnp.int32, (8, 128), 1) == 127
        LS = [slice(128*q, 128*q+128) for q in range(NQ)]
        def shl(rl, q):
            return jnp.where(first_, rl[q-1] if q > 0 else 0.0, rl[q])
        def shr(rr, q):
            return jnp.where(last_, rr[q+1] if q < NQ-1 else 0.0, rr[q])
        crow = jnp.concatenate([(lax.broadcasted_iota(jnp.int32, (8, W), 0) < 2).astype(f32), jnp.zeros((24, W), f32)], axis=0)

        class V:
            def __init__(s, src, n, za, zb, zc):
                s.src, s.n, s.za, s.zb, s.zc = src, n, za, zb, zc
                s.st = {}; s.s1 = [None]*NQ; s.done = 0; s.lastv = None; s.pend = []
            def wt(s, t, rs):
                return vs[s.za + iW + t // 4, rs, 128*(t % 4):128*(t % 4)+128]
            def U(s, g):
                rs = slice(8*g, 8*g+8)
                sl = s.n % NS
                for ls in LS:
                    vs[s.za + iXC + sl, rs, ls] = s.src[rs, ls].astype(f32)
                if form == 'P':
                    v = [vs[s.zb + iXC + sl, rs, ls] for ls in LS]
                    s.lastv = v[0]
                    s.st[g] = (v, [pltpu.roll(t, 1, 1) for t in v], [pltpu.roll(t, 127, 1) for t in v])
            def rows(s, g):
                rs = slice(8*g, 8*g+8)
                return [[vs[s.za + iXC + (s.n - 2 + i) % NS, rs, ls] for ls in LS] for i in range(3)]
            def D(s, g):
                rs = slice(8*g, 8*g+8)
                x = s.rows(g)
                A = []
                for j in ((0, 2) if not hold else (0, 2, 1)):
                    w = [s.wt(3*i+j, rs) for i in range(3)]
                    A.append([x[0][q]*w[0] + x[1][q]*w[1] + x[2][q]*w[2] for q in range(NQ)])
                s.lastv = A[1][0]
                s.st[g] = ([pltpu.roll(t, 1, 1) for t in A[0]], [pltpu.roll(t, 127, 1) for t in A[1]], A[2] if hold else None)
            def Cc(s, g):
                rs = slice(8*g, 8*g+8)
                if form == 'P':
                    v, rl, rr = s.st.pop(g)
                    if not hold:
                        v = [vs[s.za + iXC + s.n % NS, rs, ls] for ls in LS]
                    w = [s.wt(t, rs) for t in range(9)]
                    p0 = [vs[s.za + iP0, rs, ls] for ls in LS]
                    p1 = [vs[s.za + iP1, rs, ls] for ls in LS]
                    for q in range(NQ):
                        xl = shl(rl, q); xr = shr(rr, q)
                        T = [xl*w[3*i] + v[q]*w[3*i+1] + xr*w[3*i+2] for i in range(3)]
                        o = p0[q] + T[2]
                        s.pend += [(iP0, rs, q, p1[q] + T[1]), (iP1, rs, q, T[0]), (iCV, rs, q, o)]
                        s.s1[q] = o if s.s1[q] is None else s.s1[q] + o
                else:
                    rl, rr, A1 = s.st.pop(g)
                    if not hold:
                        x = [[vs[s.zb + iXC + (s.n - 2 + i) % NS, rs, ls] for ls in LS] for i in range(3)]
                        w = [s.wt(3*i+1, rs) for i in range(3)]
                        A1 = [x[0][q]*w[0] + x[1][q]*w[1] + x[2][q]*w[2] for q in range(NQ)]
                    for q in range(NQ):
                        o = (shl(rl, q) + shr(rr, q)) + A1[q]
                        s.pend.append((iCV, rs, q, o))
                        s.s1[q] = o if s.s1[q] is None else s.s1[q] + o
                s.lastv = o
                s.done += 1
                if s.done == C//8:
                    for q in range(NQ):
                        s.pend.append((iS1, slice(0, 8), q, s.s1[q]))
            def flush(s):
                for i, rs, q, val in s.pend:
                    vs[s.za + i, rs, LS[q]] = val
                s.pend = []
            def LN(s, q):
                ls = LS[q]
                q = {0:0,1:1,2:2,3:3}[q]
                s.s1load()[q] = vs[s.za + iS1, 0:8, ls]
                m = jnp.sum(s.s1load()[q], axis=0, keepdims=True) * (1.0/C)
                d = [vs[s.za + iCV, 8*g:8*g+8, ls] - m for g in range(C//8)]
                v = d[0]*d[0]
                for t in d[1:]:
                    v = v + t*t
                v = jnp.sum(v, axis=0, keepdims=True) * (1.0/C)
                r = lax.rsqrt(v + EPS) * S_
                for g in range(C//8):
                    vs[s.za + iXN, 8*g:8*g+8, ls] = d[g] * r
            def s1load(s):
                if not hasattr(s, 's1v'):
                    s.s1v = {}
                return s.s1v
            def tok(s):
                vs[s.zc + iTOK, 0:8, 0:128] = s.lastv

        def row(prog, vcur, vprev, vnext, slot, dst, za, zb, zc, xnv, isfirst, islast):
            marks = {(op, i) for op, i in prog if op in 'wx'}
            ld = {}
            def wload(op, i):
                if (op, i) not in ld:
                    idx = i if op == 'w' else 24 + i
                    src = vs[(zc + iWT,) + wslot(idx)] if (op, i) in marks else wts[(0,) + wslot(idx)]
                    ld[(op, i)] = pltpu.bitcast(src, bf16)
                return ld[(op, i)]
            st = dict(y=None, hs=None, k=0, xnext=None)
            tv = {}
            acc = [None]*NQ
            def M1():
                wv = jnp.concatenate([wload('w', c) for c in range(24)], axis=0)
                st['y'] = y = jnp.dot(wv, jnp.concatenate([xnv, crow], axis=0), preferred_element_type=f32)
                hs = [[[] for _ in range(NQ)] for _ in range(3)]
                for c in range(24):
                    for q in range(NQ):
                        yy = y[16*c:16*c+16, LS[q]]
                        z = yy * (yy*yy + AP)
                        hh = yy * (jnp.tanh(z) + 1.0)
                        hs[c//8][q].append(hh)
                        tv[('G', c, q)] = hh[0:8]
                st['hs'] = hs
            def K(k):
                assert st['k'] == k
                st['k'] += 1
                wk = jnp.concatenate([wload('x', 6*k+g) for g in range(6)], axis=0)
                for q in range(NQ):
                    r = jnp.dot(wk, jnp.concatenate(st['hs'][k][q][::-1], axis=0), preferred_element_type=f32)
                    if not accmem:
                        acc[q] = r if k == 0 else acc[q] + r
                    elif k == 0:
                        accA[za, :, LS[q]] = r
                        acc[q] = r
                    elif k == 1:
                        acc[q] = r + accA[zb, :, LS[q]]
                        accB[za, :, LS[q]] = acc[q]
                    else:
                        acc[q] = r + accB[zb, :, LS[q]]
                    for g in range(12): tv[('ABF'[k], g, q)] = acc[q][8*g:8*g+8]
            def need(k):
                if st['y'] is None: M1()
                while st['k'] <= k: K(st['k'])
            def O(g):
                need(2)
                rs = slice(16*g, 16*g+16)
                bb = b2b[rs, :]
                for q in range(NQ):
                    fin = (acc[q][rs] + (vs[za + iXC + slot, rs, LS[q]] + bb))
                    dst[rs, LS[q]] = fin.astype(bf16)
            odone = set()
            def flush():
                vcur.flush()
                if vprev is not None: vprev.flush()
            for op, i in prog:
                if op in 'L': flush()
                if op in 'wx': wload(op, i)
                elif op in 'GABF':
                    need('GABF'.index(op) - 1)
                    vs[zc + iTOK, 0:8, 0:128] = tv[(op, i, tq)]
                    flush()
                elif op == 'W': flush()
                elif op == 'O': O(i); odone.add(i)
                elif op == 'L': vcur.LN(i)
                elif op == 'U': vcur.U(i)
                elif op == 'D': vcur.D(i)
                elif op == 'C': vcur.Cc(i)
                elif op == 'K': vcur.tok()
                elif op == 'k':
                    if not isfirst: vprev.tok()
                elif op == 'c':
                    if not isfirst: vprev.Cc(i)
                elif op == 'd':
                    if not isfirst: vprev.D(i)
                elif op == 'u':
                    if not isfirst: vprev.U(i)
                elif op == 'M':
                    if not islast: st['xnext'] = vs[za + iXN]
            for g in range(C//16):
                if g not in odone: O(g)
            if islast:
                for op, i in prog:
                    if op == 'u': vcur.U(i)
                    if op == 'd': vcur.D(i)
                    if op == 'c': vcur.Cc(i)
            flush()
            return st['xnext'] if st['xnext'] is not None else xnv

        pre.wait()
        for n in range(L):
            v = V(xpre.at[n], n, zs[0], zs[1], zs[2])
            for g in range(12): v.U(g)
            if form == 'P' or n >= 1:
                for g in range(12):
                    if form != 'P': v.D(g)
                    v.Cc(g)
                v.flush()
            if n == 1:
                for q in range(NQ): v.LN(q)

        def body(j, c):
            slot = j % 2
            @pl.when(j + 1 < NCH - 1)
            def _():
                in_copy(j+1, 1-slot).start()
            @pl.when(j + 1 == NCH - 1)
            def _():
                if R > L: in_copy_last(1-slot).start()
                xin[1-slot, R-L:R] = jnp.zeros((L, C, W), bf16)
            @pl.when(j < NCH - 1)
            def _():
                in_copy(j, slot).wait()
            if R > L:
                @pl.when(j == NCH - 1)
                def _():
                    in_copy_last(slot).wait()
            @pl.when(j >= 2)
            def _():
                out_copy(j-2, slot).wait()
            za = zs[0]; zb = zs[1]; zc = zs[2]
            xnv = vs[za + iXN]
            vprev = None
            for r in range(R):
                p = first if (r == 0 and first) else last if (r == R-1 and last) else prog
                vcur = V(xin.at[slot, r], r + 3, za, zb, zc)
                vnext = V(xin.at[slot, r], r + 4, za, zb, zc)
                xnv = row(parse(p), vcur, vprev, vnext, r % NS, obuf.at[slot, r], za, zb, zc, xnv, r == 0, r == R-1)
                vprev = vcur
            out_copy(j, slot).start()
            return c
        lax.fori_loop(0, NCH, body, 0)
        out_copy(NCH-2, 0).wait()
        out_copy(NCH-1, 1).wait()

    @jax.jit
    def f(x, dw, w1, b1, w2, b2, gamma):
        xt = jnp.transpose(x, (0, 1, 3, 2)).reshape(H, C, W)
        vm = pl.BlockSpec(memory_space=pltpu.VMEM)
        anys = pl.BlockSpec(memory_space=pl.ANY)
        out = pl.pallas_call(
            kern,
            in_specs=[anys, vm, vm, vm, vm, vm, vm],
            out_specs=anys,
            out_shape=jax.ShapeDtypeStruct((H, C, W), bf16),
            scratch_shapes=[pltpu.VMEM((2, R, C, W), bf16), pltpu.VMEM((L, C, W), bf16), pltpu.VMEM((2, R, C, W), bf16),
                            pltpu.VMEM((14, C, W), f32), pltpu.VMEM((1, C, W), f32), pltpu.VMEM((1, C, W), f32), pltpu.VMEM((1, C, W), f32),
                            pltpu.VMEM((C, 128), f32), pltpu.SMEM((4,), jnp.int32),
                            pltpu.SemaphoreType.DMA((2,)), pltpu.SemaphoreType.DMA((2,)), pltpu.SemaphoreType.DMA(())],
            compiler_params=pltpu.CompilerParams(vmem_limit_bytes=64*1024*1024, flags=flags),
        )(xt, dw.reshape(9, C), w1, b1.reshape(1, E), w2.T, b2.reshape(1, C), gamma.reshape(1, C))
        return jnp.transpose(out.reshape(1, H, C, W), (0, 1, 3, 2))
    return f


def RP(L, Cs, Ds, M, extra=()):
    ev = []
    for g in range(12):
        if Ds is not None:
            ev.append((Ds[g], f"U{g} D{g}") if Ds[g] < 672 else (Ds[g]-672, f"u{g} d{g}"))
        ev.append((Cs[g], f"C{g}") if Cs[g] < 672 else (Cs[g]-672, f"c{g}"))
    ev = sorted(ev, key=lambda e: e[0])
    ev += [(L[q], f"L{i}") for i, q in enumerate(range(4))] + [(M, "M")] + list(extra)
    return build(events=ev)


_PROG = ("G0 L0 L1 G10 L2 L3 M x5 U0 D0 U1 D1 G23 U2 D2 U3 D3 U4 D4 C0 U5 D5 C1 x14 U6 D6 C2 U7 D7 C3 x17 "
         "U8 D8 C4 U9 D9 C5 U10 D10 U11 D11 C6 C7 C8 C9 C10 C11")
_impl = make(_PROG, flags={"XLA_TPU_FORCE_LP_LLO_SCHEDULER": True})


@jax.jit
def pallas_standalone__modern_conv_block_convnext__vision_kernel(x, dw, w1, b1, w2, b2, gamma):
    return _impl(x, dw, w1, b1, w2, b2, gamma)
```

```python
import functools, contextlib
import jax, jax.numpy as jnp, numpy as np
from jax import lax
from jax.experimental import pallas as pl
from jax.experimental.pallas import tpu as pltpu

A_ = float(np.sqrt(2.0/np.pi)); B_ = A_*0.044715
S_ = B_ ** (1.0/3.0)
AP = A_/S_
EPS = 1e-5
H = W = 512; C = 96; E = 384; NQ = 4
f32 = jnp.float32; bf16 = jnp.bfloat16; u32 = jnp.uint32

def seq(a, n=12, off=0): return ' '.join(f"{a}{g}" for g in range(off, off+n))

def make(prog, first=None, last=None, R=4, form='R', accmem=True, hold=False, flags=None, tqs=(3,), onepass=False, autoU=True, nc=False, sb=False):
    NCH = H // R
    NS = 4
    L = 3
    assert R % NS == 0 and R >= L
    def parse(p):
        out = []
        for t in p.split():
            op, i = t[0], int(t[1:]) if len(t) > 1 else 0
            if op in 'DdE':
                ahead = autoU if autoU is not True else 0
                if i == 0:
                    for g in range(ahead): out.append(('U' if op in 'DE' else 'u', g))
                if i + ahead < 12: out.append(('U' if op in 'DE' else 'u', i + ahead))
            out.append((op, i))
        return out
    iP0, iP1, iXC, iCV, iS1, iW, iTOK, iXN, iWT = 0, 1, 2, 6, 7, 8, 11, 12, 13
    def kern(x_hbm, dw_ref, w1_ref, b1_ref, w2t_ref, b2_ref, g_ref, o_hbm,
             xin, xpre, obuf, vs, wts, accA, accB, b2b, zs, isem, osem, psem):
        def in_copy(j, slot):
            return pltpu.make_async_copy(x_hbm.at[pl.ds(j*R+L, R)], xin.at[slot], isem.at[slot])
        def in_copy_last(slot):
            return pltpu.make_async_copy(x_hbm.at[pl.ds(H-R+L, R-L)], xin.at[slot, pl.ds(0, R-L)], isem.at[slot])
        def out_copy(j, slot):
            return pltpu.make_async_copy(obuf.at[slot], o_hbm.at[pl.ds(j*R, R)], osem.at[slot])
        pre = pltpu.make_async_copy(x_hbm.at[pl.ds(0, L)], xpre, psem)
        pre.start()
        in_copy(0, 0).start()
        zs[0] = 0; zs[1] = 0; zs[2] = 0

        def bcast(row):
            r = jnp.concatenate([row, jnp.zeros((1, 32), f32)], axis=1)
            return jnp.broadcast_to(r, (128, 128)).T[:C]
        dw = dw_ref[...].astype(f32)
        for t in range(9):
            vs[iW + t // 4, :, 128*(t % 4):128*(t % 4)+128] = bcast(dw[t:t+1])
        gb = bcast(g_ref[...].astype(f32))
        b2b[...] = gb * bcast(b2_ref[...].astype(f32))
        w1 = w1_ref[...].astype(f32)
        b1 = b1_ref[...].astype(f32) * S_
        hi = b1.astype(bf16).astype(f32)
        cs = -jnp.sum(w1, axis=0, keepdims=True)
        ch = cs.astype(bf16).astype(f32)
        w1e = jnp.concatenate([w1, hi, b1 - hi, ch, cs - ch, jnp.zeros((28, E), f32)], axis=0).T
        def wslot(i): return (slice(8*(i//4), 8*(i//4)+8), slice(128*(i%4), 128*(i%4)+128))
        for k in range(3):
            for c in range(8):
                wts[(0,) + wslot(8*k+c)] = pltpu.bitcast(w1e[128*k+16*(7-c):128*k+16*(8-c)].astype(bf16), f32)
                vs[(iWT,) + wslot(8*k+c)] = pltpu.bitcast(w1e[128*k+16*(7-c):128*k+16*(8-c)].astype(bf16), f32)
        w2 = (w2t_ref[...].astype(f32) * (jnp.concatenate([gb]*3, axis=1) * (0.5/S_)))
        for k in range(3):
            for g in range(6):
                wts[(0,) + wslot(24+6*k+g)] = pltpu.bitcast(w2[16*g:16*g+16, 128*k:128*k+128].astype(bf16), f32)
                vs[(iWT,) + wslot(24+6*k+g)] = pltpu.bitcast(w2[16*g:16*g+16, 128*k:128*k+128].astype(bf16), f32)
        for i in [iP0, iP1] + [iXC+s for s in range(NS)] + [iTOK]:
            vs[i] = jnp.zeros((C, W), f32)

        first_ = lax.broadcasted_iota(jnp.int32, (8, 128), 1) == 0
        last_ = lax.broadcasted_iota(jnp.int32, (8, 128), 1) == 127
        LS = [slice(128*q, 128*q+128) for q in range(NQ)]
        def shl(rl, q):
            return jnp.where(first_, rl[q-1] if q > 0 else 0.0, rl[q])
        def shr(rr, q):
            return jnp.where(last_, rr[q+1] if q < NQ-1 else 0.0, rr[q])
        crow = jnp.concatenate([(lax.broadcasted_iota(jnp.int32, (8, W), 0) < 2).astype(f32), jnp.zeros((24, W), f32)], axis=0)

        def loadx(za):
            if nc: return jnp.concatenate([vs[za + iXN], vs[za + iS1, 16:24, :], jnp.zeros((24, W), f32)], axis=0)
            return jnp.concatenate([vs[za + iXN], crow], axis=0)
        class V:
            def __init__(s, src, n, za, zb, zc):
                s.src, s.n, s.za, s.zb, s.zc = src, n, za, zb, zc
                s.st = {}; s.s1 = [None]*NQ; s.s2 = [None]*NQ; s.done = 0; s.lastv = None; s.pend = []
            def wt(s, t, rs):
                return vs[s.za + iW + t // 4, rs, 128*(t % 4):128*(t % 4)+128]
            def U(s, g):
                rs = slice(8*g, 8*g+8)
                sl = s.n % NS
                for ls in LS:
                    vs[s.za + iXC + sl, rs, ls] = s.src[rs, ls].astype(f32)
                if form == 'P':
                    v = [vs[s.zb + iXC + sl, rs, ls] for ls in LS]
                    s.lastv = v[0]
                    s.st[g] = (v, [pltpu.roll(t, 1, 1) for t in v], [pltpu.roll(t, 127, 1) for t in v])
            def rows(s, g):
                rs = slice(8*g, 8*g+8)
                return [[vs[s.za + iXC + (s.n - 2 + i) % NS, rs, ls] for ls in LS] for i in range(3)]
            def D(s, g):
                rs = slice(8*g, 8*g+8)
                x = s.rows(g)
                A = []
                for j in ((0, 2) if not hold else (0, 2, 1)):
                    w = [s.wt(3*i+j, rs) for i in range(3)]
                    A.append([x[0][q]*w[0] + x[1][q]*w[1] + x[2][q]*w[2] for q in range(NQ)])
                s.lastv = A[1][0]
                s.st[g] = ([pltpu.roll(t, 1, 1) for t in A[0]], [pltpu.roll(t, 127, 1) for t in A[1]], A[2] if hold else None)
            def part(s, g, j):
                rs = slice(8*g, 8*g+8)
                w = [s.wt(3*i+j, rs) for i in range(3)]
                zz = s.za
                x = [[vs[zz + iXC + (s.n - 2 + i) % NS, rs, ls] for ls in LS] for i in range(3)]
                A = [x[0][q]*w[0] + x[1][q]*w[1] + x[2][q]*w[2] for q in range(NQ)]
                cur = list(s.st.get(g, (None, None, None)))
                if j == 0: cur[0] = [pltpu.roll(t, 1, 1) for t in A]
                elif j == 2: cur[1] = [pltpu.roll(t, 127, 1) for t in A]
                else: cur[2] = A
                s.st[g] = cur
            def Cc(s, g):
                rs = slice(8*g, 8*g+8)
                if form == 'P':
                    v, rl, rr = s.st.pop(g)
                    if not hold:
                        v = [vs[s.za + iXC + s.n % NS, rs, ls] for ls in LS]
                    w = [s.wt(t, rs) for t in range(9)]
                    p0 = [vs[s.za + iP0, rs, ls] for ls in LS]
                    p1 = [vs[s.za + iP1, rs, ls] for ls in LS]
                    for q in range(NQ):
                        xl = shl(rl, q); xr = shr(rr, q)
                        T = [xl*w[3*i] + v[q]*w[3*i+1] + xr*w[3*i+2] for i in range(3)]
                        o = p0[q] + T[2]
                        s.pend += [(iP0, rs, q, p1[q] + T[1]), (iP1, rs, q, T[0]), (iCV, rs, q, o)]
                        s.s1[q] = o if s.s1[q] is None else s.s1[q] + o
                else:
                    rl, rr, A1 = s.st.pop(g)
                    if A1 is None:
                        x = [[vs[s.zb + iXC + (s.n - 2 + i) % NS, rs, ls] for ls in LS] for i in range(3)]
                        w = [s.wt(3*i+1, rs) for i in range(3)]
                        A1 = [x[0][q]*w[0] + x[1][q]*w[1] + x[2][q]*w[2] for q in range(NQ)]
                    for q in range(NQ):
                        o = (shl(rl, q) + shr(rr, q)) + A1[q]
                        s.pend.append((iCV, rs, q, o))
                        s.s1[q] = o if s.s1[q] is None else s.s1[q] + o
                        if onepass: s.s2[q] = o*o if s.s2[q] is None else s.s2[q] + o*o
                s.lastv = o
                s.done += 1
                if s.done == C//8:
                    for q in range(NQ):
                        s.pend.append((iS1, slice(0, 8), q, s.s1[q]))
                        if onepass: s.pend.append((iS1, slice(8, 16), q, s.s2[q]))
            def flush(s):
                for i, rs, q, val in s.pend:
                    vs[s.za + i, rs, LS[q]] = val
                s.pend = []
            def stats4(s):
                sub = lax.broadcasted_iota(jnp.int32, (8, 128), 0)
                m4 = sub < 4
                m2 = (sub & 2) == 0
                def red(off):
                    x = [vs[s.za + iS1, off:off+8, LS[q]] for q in range(NQ)]
                    ab = jnp.where(m4, x[0], x[1]) + pltpu.roll(jnp.where(m4, x[1], x[0]), 4, 0)
                    cd = jnp.where(m4, x[2], x[3]) + pltpu.roll(jnp.where(m4, x[3], x[2]), 4, 0)
                    u = ab + pltpu.roll(ab, 6, 0)
                    w = cd + pltpu.roll(cd, 2, 0)
                    t = jnp.where(m2, u, w)
                    return (t + pltpu.roll(t, 7, 0)) * (1.0/C)
                m = red(0)
                v = jnp.maximum(red(8) - m*m, 0.0)
                r = lax.rsqrt(v + EPS) * S_
                s.sb = (m, r, m*r)
            def LN(s, q):
                ls = LS[q]
                if sb:
                    if not hasattr(s, 'sb'): s.stats4()
                    k = [0, 4, 2, 6][q]
                    bc = lambda t: jnp.broadcast_to(t[k:k+1, :], (8, 128))
                    r = bc(s.sb[1])
                    m = None if nc else bc(s.sb[0])
                    mr = bc(s.sb[2]) if nc else None
                else:
                    m = jnp.sum(vs[s.za + iS1, 0:8, ls], axis=0, keepdims=True) * (1.0/C)
                    if onepass:
                        v = jnp.maximum(jnp.sum(vs[s.za + iS1, 8:16, ls], axis=0, keepdims=True) * (1.0/C) - m*m, 0.0)
                    else:
                        d = [vs[s.za + iCV, 8*g:8*g+8, ls] - m for g in range(C//8)]
                        v0 = d[0]*d[0]; v1 = d[1]*d[1]
                        for t in d[2::2]: v0 = v0 + t*t
                        for t in d[3::2]: v1 = v1 + t*t
                        v = jnp.sum(v0 + v1, axis=0, keepdims=True) * (1.0/C)
                    r = lax.rsqrt(v + EPS) * S_
                    mr = jnp.broadcast_to(m * r, (8, 128))
                for g in range(C//8):
                    c_ = vs[s.za + iCV, 8*g:8*g+8, ls]
                    vs[s.za + iXN, 8*g:8*g+8, ls] = (c_ if nc else c_ - m) * r
                if nc:
                    sub = lax.broadcasted_iota(jnp.int32, (8, 128), 0)
                    vs[s.za + iS1, 16:24, ls] = jnp.where(sub < 2, 1.0, mr)
            def s1load(s):
                if not hasattr(s, 's1v'):
                    s.s1v = {}
                return s.s1v
            def tok(s):
                vs[s.zc + iTOK, 0:8, 0:128] = s.lastv

        def row(prog, vcur, vprev, vnext, slot, dst, za, zb, zc, xnv, isfirst, islast):
            marks = {(op, i) for op, i in prog if op in 'wx'}
            ld = {}
            def wload(op, i):
                if (op, i) not in ld:
                    idx = i if op == 'w' else 24 + i
                    src = vs[(zc + iWT,) + wslot(idx)] if (op, i) in marks else wts[(0,) + wslot(idx)]
                    ld[(op, i)] = pltpu.bitcast(src, bf16)
                return ld[(op, i)]
            st = dict(y=None, hs=None, k=0, xnext=None)
            tv = {}
            acc = [None]*NQ
            def M1():
                wv = jnp.concatenate([wload('w', c) for c in range(24)], axis=0)
                st['y'] = y = jnp.dot(wv, xnv, preferred_element_type=f32)
                hs = [[[] for _ in range(NQ)] for _ in range(3)]
                for c in range(24):
                    for q in range(NQ):
                        yy = y[16*c:16*c+16, LS[q]]
                        z = yy * (yy*yy + AP)
                        hh = yy * (jnp.tanh(z) + 1.0)
                        hs[c//8][q].append(hh)
                        tv[('G', c, q)] = hh[0:8]
                st['hs'] = hs
            def K(k):
                assert st['k'] == k
                st['k'] += 1
                wk = jnp.concatenate([wload('x', 6*k+g) for g in range(6)], axis=0)
                for q in range(NQ):
                    r = jnp.dot(wk, jnp.concatenate(st['hs'][k][q][::-1], axis=0), preferred_element_type=f32)
                    if not accmem:
                        acc[q] = r if k == 0 else acc[q] + r
                    elif k == 0:
                        accA[za, :, LS[q]] = r
                        acc[q] = r
                    elif k == 1:
                        acc[q] = r + accA[zb, :, LS[q]]
                        accB[za, :, LS[q]] = acc[q]
                    else:
                        acc[q] = r + accB[zb, :, LS[q]]
                    for g in range(12): tv[('ABF'[k], g, q)] = acc[q][8*g:8*g+8]
            def need(k):
                if st['y'] is None: M1()
                while st['k'] <= k: K(st['k'])
            def O(g):
                need(2)
                rs = slice(16*g, 16*g+16)
                bb = b2b[rs, :]
                for q in range(NQ):
                    fin = (acc[q][rs] + (vs[za + iXC + slot, rs, LS[q]] + bb))
                    dst[rs, LS[q]] = fin.astype(bf16)
            odone = set()
            def flush():
                vcur.flush()
                if vprev is not None: vprev.flush()
            for op, i in prog:
                if op in 'LS': flush()
                if op in 'wx': wload(op, i)
                elif op in 'GABF':
                    need('GABF'.index(op) - 1)
                    for q in tqs: vs[zc + iTOK, 8*q:8*q+8, 0:128] = tv[(op, i, q)]
                    flush()
                elif op == 'W': flush()
                elif op == 'O': O(i); odone.add(i)
                elif op == 'L': vcur.LN(i)
                elif op == 'U': vcur.U(i)
                elif op == 'D': vcur.D(i)
                elif op == 'C': vcur.Cc(i)
                elif op == 'E': vcur.part(i, 0)
                elif op == 'H': vcur.part(i, 2)
                elif op == 'I': vcur.part(i, 1)
                elif op == 'S': vcur.stats4()
                elif op == 'K': vcur.tok()
                elif op == 'k':
                    if not isfirst: vprev.tok()
                elif op == 'c':
                    if not isfirst: vprev.Cc(i)
                elif op == 'd':
                    if not isfirst: vprev.D(i)
                elif op == 'u':
                    if not isfirst: vprev.U(i)
                elif op == 'M':
                    if not islast: st['xnext'] = loadx(za)
            for g in range(C//16):
                if g not in odone: O(g)
            if islast:
                for op, i in prog:
                    if op == 'u': vcur.U(i)
                    if op == 'd': vcur.D(i)
                    if op == 'c': vcur.Cc(i)
            flush()
            return st['xnext'] if st['xnext'] is not None else xnv

        pre.wait()
        for n in range(L):
            v = V(xpre.at[n], n, zs[0], zs[1], zs[2])
            for g in range(12): v.U(g)
            if form == 'P' or n >= 1:
                for g in range(12):
                    if form != 'P': v.D(g)
                    v.Cc(g)
                v.flush()
            if n == 1:
                for q in range(NQ): v.LN(q)

        def body(j, c):
            slot = j % 2
            @pl.when(j + 1 < NCH - 1)
            def _():
                in_copy(j+1, 1-slot).start()
            @pl.when(j + 1 == NCH - 1)
            def _():
                if R > L: in_copy_last(1-slot).start()
                xin[1-slot, R-L:R] = jnp.zeros((L, C, W), bf16)
            @pl.when(j < NCH - 1)
            def _():
                in_copy(j, slot).wait()
            if R > L:
                @pl.when(j == NCH - 1)
                def _():
                    in_copy_last(slot).wait()
            @pl.when(j >= 2)
            def _():
                out_copy(j-2, slot).wait()
            za = zs[0]; zb = zs[1]; zc = zs[2]
            xnv = loadx(za)
            vprev = None
            for r in range(R):
                p = first if (r == 0 and first) else last if (r == R-1 and last) else prog
                vcur = V(xin.at[slot, r], r + 3, za, zb, zc)
                vnext = V(xin.at[slot, r], r + 4, za, zb, zc)
                xnv = row(parse(p), vcur, vprev, vnext, r % NS, obuf.at[slot, r], za, zb, zc, xnv, r == 0, r == R-1)
                vprev = vcur
            out_copy(j, slot).start()
            return c
        lax.fori_loop(0, NCH, body, 0)
        out_copy(NCH-2, 0).wait()
        out_copy(NCH-1, 1).wait()

    @jax.jit
    def f(x, dw, w1, b1, w2, b2, gamma):
        xt = jnp.transpose(x, (0, 1, 3, 2)).reshape(H, C, W)
        vm = pl.BlockSpec(memory_space=pltpu.VMEM)
        anys = pl.BlockSpec(memory_space=pl.ANY)
        out = pl.pallas_call(
            kern,
            in_specs=[anys, vm, vm, vm, vm, vm, vm],
            out_specs=anys,
            out_shape=jax.ShapeDtypeStruct((H, C, W), bf16),
            scratch_shapes=[pltpu.VMEM((2, R, C, W), bf16), pltpu.VMEM((L, C, W), bf16), pltpu.VMEM((2, R, C, W), bf16),
                            pltpu.VMEM((14, C, W), f32), pltpu.VMEM((1, C, W), f32), pltpu.VMEM((1, C, W), f32), pltpu.VMEM((1, C, W), f32),
                            pltpu.VMEM((C, 128), f32), pltpu.SMEM((4,), jnp.int32),
                            pltpu.SemaphoreType.DMA((2,)), pltpu.SemaphoreType.DMA((2,)), pltpu.SemaphoreType.DMA(())],
            compiler_params=pltpu.CompilerParams(vmem_limit_bytes=64*1024*1024, flags=flags),
        )(xt, dw.reshape(9, C), w1, b1.reshape(1, E), w2.T, b2.reshape(1, C), gamma.reshape(1, C))
        return jnp.transpose(out.reshape(1, H, C, W), (0, 1, 3, 2))
    return f


_CFG = {'prog': 'L0 G0 L1 G5 L2 G10 L3 D0 x8 G16 G19 D1 G20 D2 G22 D3 D4 D5 C0 D6 D7 M C1 D8 C2 C3 D9 C4 C5 D10 C6 C7 x11 D11 C8 C9 C10 C11 O0 O1 O2 O3 O4 O5', 'first': 'L0 L3 L1 L2 G10 D0 x3 D1 G13 D2 G22 D3 D4 D5 C0 D6 D7 M C1 D8 C2 C3 D9 C4 C5 D10 C6 C7 D11 C8 C9 C10 C11 O0 O1 O2 O3 O4 O5', 'last': 'L0 G0 L1 G5 L2 G10 L3 D0 x11 D1 G20 D2 G22 D3 G23 D4 D5 C0 D6 D7 M C1 D8 C2 C3 D9 C4 C5 D10 C6 C7 D11 C8 C9 C10 C11 O0 O1 O2 O3 O4 O5', 'autoU': 3, 'hold': True, 'accmem': True, 'tqs': (0,), 'sb': False, 'nc': True}
_impl = make(R=8, onepass=True, flags={"XLA_TPU_FORCE_LP_LLO_SCHEDULER": True}, **_CFG)


@jax.jit
def pallas_standalone__modern_conv_block_convnext__vision_kernel(x, dw, w1, b1, w2, b2, gamma):
    return _impl(x, dw, w1, b1, w2, b2, gamma)
```

```python
import functools, contextlib
import jax, jax.numpy as jnp, numpy as np
from jax import lax
from jax.experimental import pallas as pl
from jax.experimental.pallas import tpu as pltpu

A_ = float(np.sqrt(2.0/np.pi)); B_ = A_*0.044715
S_ = B_ ** (1.0/3.0)
AP = A_/S_
EPS = 1e-5
H = W = 512; C = 96; E = 384; NQ = 4
f32 = jnp.float32; bf16 = jnp.bfloat16; u32 = jnp.uint32

def seq(a, n=12, off=0): return ' '.join(f"{a}{g}" for g in range(off, off+n))

def make(prog, osplit=1, NROWS=512, man=(), first=None, last=None, R=4, form='R', accmem=True, hold=False, flags=None, tqs=(3,), onepass=False, autoU=True, nc=False, sb=False):
    NCH = NROWS // R
    NS = 4
    L = 3
    assert R % NS == 0 and R >= L
    def parse(p):
        out = []; nu = {'U': 0, 'u': 0}
        for t in p.split():
            op, i = t[0], int(t[1:]) if len(t) > 1 else 0
            if op in 'DdEHIJ':
                g = i // 6 if op == 'J' else i
                k = 'u' if op == 'd' else 'U'
                while nu[k] < min(12, g + 1 + autoU):
                    out.append((k, nu[k])); nu[k] += 1
            out.append((op, i))
        return out
    iP0, iP1, iXC, iCV, iS1, iW, iTOK, iXN, iWT = 0, 1, 2, 6, 7, 8, 11, 12, 13
    def kern(x_hbm, dw_h, w1_h, b1_h, w2t_h, b2_h, g_h, o_hbm, dw_ref, w1_ref, b1_ref, w2t_ref, b2_ref, g_ref, wsem,
             xin, xpre, obuf, vs, wts, accA, accB, b2b, zs, isem, osem, psem):
        def in_copy(j, slot):
            return pltpu.make_async_copy(x_hbm.at[pl.ds(j*R+L, R)], xin.at[slot], isem.at[slot])
        def in_copy_last(slot):
            return pltpu.make_async_copy(x_hbm.at[pl.ds(H-R+L, R-L)], xin.at[slot, pl.ds(0, R-L)], isem.at[slot])
        RS_ = R // osplit
        class OC:
            def __init__(s, j, slot): s.j, s.slot = j, slot
            def part(s, p): return pltpu.make_async_copy(obuf.at[s.slot, pl.ds(p*RS_, RS_)], o_hbm.at[pl.ds(s.j*R + p*RS_, RS_)], osem.at[s.slot, p])
            def wait(s):
                for p in range(osplit): s.part(p).wait()
        out_copy = OC
        pre = pltpu.make_async_copy(x_hbm.at[pl.ds(0, L)], xpre, psem)
        pre.start()
        class Nop:
            def start(s): pass
            def wait(s): pass
        wc = {n: (pltpu.make_async_copy(a, b, wsem.at[i]) if n in man else Nop()) for i, (n, a, b) in enumerate([
            ('dw', dw_h, dw_ref), ('g', g_h, g_ref), ('b2', b2_h, b2_ref), ('w1', w1_h, w1_ref), ('b1', b1_h, b1_ref), ('w2', w2t_h, w2t_ref)])}
        for cp in wc.values(): cp.start()
        if 'dw' not in man: dw_ref = dw_h
        if 'g' not in man: g_ref = g_h
        if 'b2' not in man: b2_ref = b2_h
        if 'w1' not in man: w1_ref = w1_h
        if 'b1' not in man: b1_ref = b1_h
        if 'w2' not in man: w2t_ref = w2t_h
        zs[0] = 0; zs[1] = 0; zs[2] = 0

        in_copy(0, 0).start()
        def bcast(row):
            r = jnp.concatenate([row, jnp.zeros((1, 32), f32)], axis=1)
            return jnp.broadcast_to(r, (128, 128)).T[:C]
        for i in [iXC+NS-1]:
            vs[i] = jnp.zeros((C, W), f32)
        wc['dw'].wait()
        for t in range(9):
            vs[iW + t // 4, :, 128*(t % 4):128*(t % 4)+128] = bcast(dw_ref[t // 3].astype(f32)[t % 3:t % 3+1])
        wc['g'].wait(); wc['b2'].wait()
        gb = bcast(g_ref[...].astype(f32).reshape(1, C))
        b2b[...] = gb * bcast(b2_ref[...].astype(f32).reshape(1, C))
        wc['w1'].wait(); wc['b1'].wait(); wc['w2'].wait()
        w1 = w1_ref[...].astype(f32)
        b1 = b1_ref[...].astype(f32).reshape(1, E) * S_
        hi = b1.astype(bf16).astype(f32)
        cs = -jnp.sum(w1, axis=0, keepdims=True)
        ch = cs.astype(bf16).astype(f32)
        w1e = jnp.concatenate([w1, hi, b1 - hi, ch, cs - ch, jnp.zeros((28, E), f32)], axis=0).T
        def wslot(i): return (slice(8*(i//4), 8*(i//4)+8), slice(128*(i%4), 128*(i%4)+128))
        for k in range(3):
            for c in range(8):
                wts[(0,) + wslot(8*k+c)] = pltpu.bitcast(w1e[128*k+16*(7-c):128*k+16*(8-c)].astype(bf16), f32)
                vs[(iWT,) + wslot(8*k+c)] = pltpu.bitcast(w1e[128*k+16*(7-c):128*k+16*(8-c)].astype(bf16), f32)
        w2 = (w2t_ref[...].astype(f32) * (jnp.concatenate([gb]*3, axis=1) * (0.5/S_)))
        for k in range(3):
            for g in range(6):
                wts[(0,) + wslot(24+6*k+g)] = pltpu.bitcast(w2[16*g:16*g+16, 128*k:128*k+128].astype(bf16), f32)
                vs[(iWT,) + wslot(24+6*k+g)] = pltpu.bitcast(w2[16*g:16*g+16, 128*k:128*k+128].astype(bf16), f32)

        first_ = lax.broadcasted_iota(jnp.int32, (8, 128), 1) == 0
        last_ = lax.broadcasted_iota(jnp.int32, (8, 128), 1) == 127
        LS = [slice(128*q, 128*q+128) for q in range(NQ)]
        def shl(rl, q):
            return jnp.where(first_, rl[q-1] if q > 0 else 0.0, rl[q])
        def shr(rr, q):
            return jnp.where(last_, rr[q+1] if q < NQ-1 else 0.0, rr[q])
        crow = jnp.concatenate([(lax.broadcasted_iota(jnp.int32, (8, W), 0) < 2).astype(f32), jnp.zeros((24, W), f32)], axis=0)

        def loadx(za):
            if nc: return jnp.concatenate([vs[za + iXN], vs[za + iS1, 16:24, :], jnp.zeros((24, W), f32)], axis=0)
            return jnp.concatenate([vs[za + iXN], crow], axis=0)
        class V:
            def __init__(s, src, n, za, zb, zc):
                s.src, s.n, s.za, s.zb, s.zc = src, n, za, zb, zc
                s.st = {}; s.s1 = [None]*NQ; s.s2 = [None]*NQ; s.done = 0; s.lastv = None; s.pend = []
            def wt(s, t, rs):
                return vs[s.za + iW + t // 4, rs, 128*(t % 4):128*(t % 4)+128]
            def U(s, g):
                rs = slice(8*g, 8*g+8)
                sl = s.n % NS
                for ls in LS:
                    vs[s.za + iXC + sl, rs, ls] = s.src[rs, ls].astype(f32)
                if form == 'P':
                    v = [vs[s.zb + iXC + sl, rs, ls] for ls in LS]
                    s.lastv = v[0]
                    s.st[g] = (v, [pltpu.roll(t, 1, 1) for t in v], [pltpu.roll(t, 127, 1) for t in v])
            def rows(s, g):
                rs = slice(8*g, 8*g+8)
                return [[vs[s.za + iXC + (s.n - 2 + i) % NS, rs, ls] for ls in LS] for i in range(3)]
            def D(s, g):
                rs = slice(8*g, 8*g+8)
                x = s.rows(g)
                A = []
                for j in ((0, 2) if not hold else (0, 2, 1)):
                    w = [s.wt(3*i+j, rs) for i in range(3)]
                    A.append([x[0][q]*w[0] + x[1][q]*w[1] + x[2][q]*w[2] for q in range(NQ)])
                s.lastv = A[1][0]
                s.st[g] = ([pltpu.roll(t, 1, 1) for t in A[0]], [pltpu.roll(t, 127, 1) for t in A[1]], A[2] if hold else None)
            def part(s, g, j):
                rs = slice(8*g, 8*g+8)
                w = [s.wt(3*i+j, rs) for i in range(3)]
                zz = s.za
                x = [[vs[zz + iXC + (s.n - 2 + i) % NS, rs, ls] for ls in LS] for i in range(3)]
                A = [x[0][q]*w[0] + x[1][q]*w[1] + x[2][q]*w[2] for q in range(NQ)]
                cur = list(s.st.get(g, (None, None, None)))
                if j == 0: cur[0] = [pltpu.roll(t, 1, 1) for t in A]
                elif j == 2: cur[1] = [pltpu.roll(t, 127, 1) for t in A]
                else: cur[2] = A
                s.st[g] = cur
            def half(s, n):
                g, j = divmod(n, 6)
                jj = (0, 2, 1, 0, 2, 1)[j]; qs = (0, 1) if j < 3 else (2, 3)
                rs = slice(8*g, 8*g+8)
                w = [s.wt(3*i+jj, rs) for i in range(3)]
                cur = [list(t) if t else [None]*NQ for t in s.st.get(g, (None, None, None))]
                for q in qs:
                    x = [vs[s.za + iXC + (s.n - 2 + i) % NS, rs, LS[q]] for i in range(3)]
                    A = x[0]*w[0] + x[1]*w[1] + x[2]*w[2]
                    if jj == 0: cur[0][q] = pltpu.roll(A, 1, 1)
                    elif jj == 2: cur[1][q] = pltpu.roll(A, 127, 1)
                    else: cur[2][q] = A
                s.st[g] = cur
            def Cc(s, g):
                rs = slice(8*g, 8*g+8)
                if form == 'P':
                    v, rl, rr = s.st.pop(g)
                    if not hold:
                        v = [vs[s.za + iXC + s.n % NS, rs, ls] for ls in LS]
                    w = [s.wt(t, rs) for t in range(9)]
                    p0 = [vs[s.za + iP0, rs, ls] for ls in LS]
                    p1 = [vs[s.za + iP1, rs, ls] for ls in LS]
                    for q in range(NQ):
                        xl = shl(rl, q); xr = shr(rr, q)
                        T = [xl*w[3*i] + v[q]*w[3*i+1] + xr*w[3*i+2] for i in range(3)]
                        o = p0[q] + T[2]
                        s.pend += [(iP0, rs, q, p1[q] + T[1]), (iP1, rs, q, T[0]), (iCV, rs, q, o)]
                        s.s1[q] = o if s.s1[q] is None else s.s1[q] + o
                else:
                    rl, rr, A1 = s.st.pop(g)
                    if A1 is None:
                        x = [[vs[s.zb + iXC + (s.n - 2 + i) % NS, rs, ls] for ls in LS] for i in range(3)]
                        w = [s.wt(3*i+1, rs) for i in range(3)]
                        A1 = [x[0][q]*w[0] + x[1][q]*w[1] + x[2][q]*w[2] for q in range(NQ)]
                    for q in range(NQ):
                        o = (shl(rl, q) + shr(rr, q)) + A1[q]
                        s.pend.append((iCV, rs, q, o))
                        s.s1[q] = o if s.s1[q] is None else s.s1[q] + o
                        if onepass: s.s2[q] = o*o if s.s2[q] is None else s.s2[q] + o*o
                s.lastv = o
                s.done += 1
                if s.done == C//8:
                    for q in range(NQ):
                        s.pend.append((iS1, slice(0, 8), q, s.s1[q]))
                        if onepass: s.pend.append((iS1, slice(8, 16), q, s.s2[q]))
            def flush(s):
                for i, rs, q, val in s.pend:
                    vs[s.za + i, rs, LS[q]] = val
                s.pend = []
            def stats4(s):
                sub = lax.broadcasted_iota(jnp.int32, (8, 128), 0)
                m4 = sub < 4
                m2 = (sub & 2) == 0
                def red(off):
                    x = [vs[s.za + iS1, off:off+8, LS[q]] for q in range(NQ)]
                    ab = jnp.where(m4, x[0], x[1]) + pltpu.roll(jnp.where(m4, x[1], x[0]), 4, 0)
                    cd = jnp.where(m4, x[2], x[3]) + pltpu.roll(jnp.where(m4, x[3], x[2]), 4, 0)
                    u = ab + pltpu.roll(ab, 6, 0)
                    w = cd + pltpu.roll(cd, 2, 0)
                    t = jnp.where(m2, u, w)
                    return (t + pltpu.roll(t, 7, 0)) * (1.0/C)
                m = red(0)
                v = jnp.maximum(red(8) - m*m, 0.0)
                r = lax.rsqrt(v + EPS) * S_
                s.sb = (m, r, m*r)
            def LN(s, q):
                ls = LS[q]
                if sb:
                    if not hasattr(s, 'sb'): s.stats4()
                    k = [0, 4, 2, 6][q]
                    bc = lambda t: jnp.broadcast_to(t[k:k+1, :], (8, 128))
                    r = bc(s.sb[1])
                    m = None if nc else bc(s.sb[0])
                    mr = bc(s.sb[2]) if nc else None
                else:
                    m = jnp.sum(vs[s.za + iS1, 0:8, ls], axis=0, keepdims=True) * (1.0/C)
                    if onepass:
                        v = jnp.maximum(jnp.sum(vs[s.za + iS1, 8:16, ls], axis=0, keepdims=True) * (1.0/C) - m*m, 0.0)
                    else:
                        d = [vs[s.za + iCV, 8*g:8*g+8, ls] - m for g in range(C//8)]
                        v0 = d[0]*d[0]; v1 = d[1]*d[1]
                        for t in d[2::2]: v0 = v0 + t*t
                        for t in d[3::2]: v1 = v1 + t*t
                        v = jnp.sum(v0 + v1, axis=0, keepdims=True) * (1.0/C)
                    r = lax.rsqrt(v + EPS) * S_
                    mr = jnp.broadcast_to(m * r, (8, 128))
                for g in range(C//8):
                    c_ = vs[s.za + iCV, 8*g:8*g+8, ls]
                    vs[s.za + iXN, 8*g:8*g+8, ls] = (c_ if nc else c_ - m) * r
                if nc:
                    sub = lax.broadcasted_iota(jnp.int32, (8, 128), 0)
                    vs[s.za + iS1, 16:24, ls] = jnp.where(sub < 2, 1.0, mr)
            def s1load(s):
                if not hasattr(s, 's1v'):
                    s.s1v = {}
                return s.s1v
            def tok(s):
                vs[s.zc + iTOK, 0:8, 0:128] = s.lastv

        def row(prog, vcur, vprev, vnext, slot, dst, za, zb, zc, xnv, isfirst, islast):
            marks = {(op, i) for op, i in prog if op in 'wx'}
            ld = {}
            def wload(op, i):
                if (op, i) not in ld:
                    idx = i if op == 'w' else 24 + i
                    src = vs[(zc + iWT,) + wslot(idx)] if (op, i) in marks else wts[(0,) + wslot(idx)]
                    ld[(op, i)] = pltpu.bitcast(src, bf16)
                return ld[(op, i)]
            st = dict(y=None, hs=None, k=0, xnext=None)
            tv = {}
            acc = [None]*NQ
            def M1():
                wv = jnp.concatenate([wload('w', c) for c in range(24)], axis=0)
                st['y'] = y = jnp.dot(wv, xnv, preferred_element_type=f32)
                hs = [[[] for _ in range(NQ)] for _ in range(3)]
                for c in range(24):
                    for q in range(NQ):
                        yy = y[16*c:16*c+16, LS[q]]
                        z = yy * (yy*yy + AP)
                        hh = yy * (jnp.tanh(z) + 1.0)
                        hs[c//8][q].append(hh)
                        tv[('G', c, q)] = hh[0:8]
                st['hs'] = hs
            def K(k):
                assert st['k'] == k
                st['k'] += 1
                wk = jnp.concatenate([wload('x', 6*k+g) for g in range(6)], axis=0)
                for q in range(NQ):
                    r = jnp.dot(wk, jnp.concatenate(st['hs'][k][q][::-1], axis=0), preferred_element_type=f32)
                    if not accmem:
                        acc[q] = r if k == 0 else acc[q] + r
                    elif k == 0:
                        accA[za, :, LS[q]] = r
                        acc[q] = r
                    elif k == 1:
                        if accmem == 2:
                            acc[q] = r
                            accB[za, :, LS[q]] = r
                        else:
                            acc[q] = r + accA[zb, :, LS[q]]
                            accB[za, :, LS[q]] = acc[q]
                    elif accmem == 2:
                        acc[q] = (r + accA[zb, :, LS[q]]) + accB[zb, :, LS[q]]
                    else:
                        acc[q] = r + accB[zb, :, LS[q]]
                    for g in range(12): tv[('ABF'[k], g, q)] = acc[q][8*g:8*g+8]
            def need(k):
                if st['y'] is None: M1()
                while st['k'] <= k: K(st['k'])
            def O(g):
                need(2)
                for gg in (2*g, 2*g+1):
                    rs = slice(8*gg, 8*gg+8)
                    bb = b2b[rs, :]
                    fin = [(acc[q][rs] + (vs[za + iXC + slot, rs, LS[q]] + bb)) for q in range(NQ)]
                    for h in range(2):
                        dst[rs, 256*h:256*h+256] = jnp.concatenate(fin[2*h:2*h+2], axis=1).astype(bf16)
            odone = set()
            def flush():
                vcur.flush()
                if vprev is not None: vprev.flush()
            for op, i in prog:
                if op in 'LS': flush()
                if op in 'wx': wload(op, i)
                elif op in 'GABF':
                    need('GABF'.index(op) - 1)
                    for q in tqs: vs[zc + iTOK, 8*q:8*q+8, 0:128] = tv[(op, i, q)]
                    flush()
                elif op == 'W': flush()
                elif op == 'O': O(i); odone.add(i)
                elif op == 'L': vcur.LN(i)
                elif op == 'U': vcur.U(i)
                elif op == 'D': vcur.D(i)
                elif op == 'C': vcur.Cc(i)
                elif op == 'E': vcur.part(i, 0)
                elif op == 'H': vcur.part(i, 2)
                elif op == 'I': vcur.part(i, 1)
                elif op == 'S': vcur.stats4()
                elif op == 'J': vcur.half(i)
                elif op == 'K': vcur.tok()
                elif op == 'k':
                    if not isfirst: vprev.tok()
                elif op == 'c':
                    if not isfirst: vprev.Cc(i)
                elif op == 'd':
                    if not isfirst: vprev.D(i)
                elif op == 'u':
                    if not isfirst: vprev.U(i)
                elif op == 'M':
                    if not islast: st['xnext'] = loadx(za)
            for g in range(C//16):
                if g not in odone: O(g)
            if islast:
                for op, i in prog:
                    if op == 'u': vcur.U(i)
                    if op == 'd': vcur.D(i)
                    if op == 'c': vcur.Cc(i)
            flush()
            return st['xnext'] if st['xnext'] is not None else xnv

        pre.wait()
        for n in range(L):
            v = V(xpre.at[n], n, zs[0], zs[1], zs[2])
            for g in range(12): v.U(g)
            if form == 'P' or n >= 1:
                for g in range(12):
                    if form != 'P': v.D(g)
                    v.Cc(g)
                v.flush()
            if n == 1:
                for q in range(NQ): v.LN(q)

        def body(j, c):
            slot = j % 2
            @pl.when(j + 1 < NCH - 1)
            def _():
                in_copy(j+1, 1-slot).start()
            @pl.when(j + 1 == NCH - 1)
            def _():
                if R > L: in_copy_last(1-slot).start()
                xin[1-slot, R-L:R] = jnp.zeros((L, C, W), bf16)
            @pl.when(j < NCH - 1)
            def _():
                in_copy(j, slot).wait()
            if R > L:
                @pl.when(j == NCH - 1)
                def _():
                    in_copy_last(slot).wait()
            @pl.when(j >= 2)
            def _():
                out_copy(j-2, slot).wait()
            za = zs[0]; zb = zs[1]; zc = zs[2]
            xnv = loadx(za)
            vprev = None
            for r in range(R):
                p = first if (r == 0 and first) else last if (r == R-1 and last) else prog
                vcur = V(xin.at[slot, r], r + 3, za, zb, zc)
                vnext = V(xin.at[slot, r], r + 4, za, zb, zc)
                xnv = row(parse(p), vcur, vprev, vnext, r % NS, obuf.at[slot, r], za, zb, zc, xnv, r == 0, r == R-1)
                vprev = vcur
                if (r + 1) % RS_ == 0: out_copy(j, slot).part((r + 1)//RS_ - 1).start()
            return c
        lax.fori_loop(0, NCH, body, 0)
        out_copy(NCH-2, 0).wait()
        out_copy(NCH-1, 1).wait()

    @jax.jit
    def f(x, dw, w1, b1, w2, b2, gamma):
        xt = jnp.transpose(x, (0, 1, 3, 2)).reshape(H, C, W)
        vm = pl.BlockSpec(memory_space=pltpu.VMEM)
        anys = pl.BlockSpec(memory_space=pl.ANY)
        out = pl.pallas_call(
            kern,
            in_specs=[anys] + [anys if n in man else vm for n in ('dw','w1','b1','w2','b2','g')],
            out_specs=anys,
            out_shape=jax.ShapeDtypeStruct((H, C, W), bf16),
            scratch_shapes=[pltpu.VMEM((3,3,C), bf16), pltpu.VMEM((C,E), bf16), pltpu.VMEM((E,), bf16), pltpu.VMEM((C,E), bf16), pltpu.VMEM((C,), bf16), pltpu.VMEM((C,), bf16), pltpu.SemaphoreType.DMA((6,)), pltpu.VMEM((2, R, C, W), bf16), pltpu.VMEM((L, C, W), bf16), pltpu.VMEM((2, R, C, W), bf16),
                            pltpu.VMEM((14, C, W), f32), pltpu.VMEM((1, C, W), f32), pltpu.VMEM((1, C, W), f32), pltpu.VMEM((1, C, W), f32),
                            pltpu.VMEM((C, 128), f32), pltpu.SMEM((4,), jnp.int32),
                            pltpu.SemaphoreType.DMA((2,)), pltpu.SemaphoreType.DMA((2, osplit)), pltpu.SemaphoreType.DMA(())],
            compiler_params=pltpu.CompilerParams(vmem_limit_bytes=64*1024*1024, flags=flags),
        )(xt, dw, w1, b1, w2.T, b2, gamma)
        return jnp.transpose(out.reshape(1, H, C, W), (0, 1, 3, 2))
    return f


_CFG = {'prog': 'L1 J0 G0 G3 L0 J2 J1 G4 J3 G5 J4 G6 L2 J5 G7 J6 G8 J7 G9 J8 G10 L3 J9 G11 J10 G12 J11 J12 G13 J13 G14 J14 G15 J15 G16 J16 G17 J19 J17 G18 J18 G19 G20 J20 G21 J21 A3 G22 J22 G23 D4 J23 D5 D6 C0 M C1 D7 C2 C3 D8 C4 C5 D9 C6 C7 D10 C8 C9 D11 C10 C11 O0 O1 O2 O3 O4 O5', 'first': 'L0 L1 L2 L3 E0 H0 G4 H1 g8 I0 E1 G12 I1 G14 g18 E2 G18 H2 G21 D3 I2 D4 D5 D6 M C0 E7 H7 I7 C1 C2 C3 D8 C4 C5 D9 C6 C7 D10 C8 C9 O0 D11 C10 C11 O1 O2 O3 O4 O5', 'last': 'L1 L0 G0 G4 L2 E0 L3 H0 G6 I0 G8 E1 I1 E2 H1 H2 I2 G20 D3 D4 D5 C0 G22 E6 H6 M C1 D7 C2 C3 A11 C4 D8 C5 D9 C6 C7 D10 C8 C9 D11 C10 C11 O0 O1 O2 O3 O4 O5', 'autoU': 0, 'hold': True, 'accmem': 2, 'tqs': (1,), 'sb': True, 'nc': True}
_impl = make(R=16, osplit=2, onepass=True, flags={"XLA_TPU_FORCE_LP_LLO_SCHEDULER": True}, **_CFG)


@jax.jit
def pallas_standalone__modern_conv_block_convnext__vision_kernel(x, dw, w1, b1, w2, b2, gamma):
    return _impl(x, dw, w1, b1, w2, b2, gamma)
```

```python
import jax
import jax.numpy as jnp
import numpy as np
from jax import lax
from jax.experimental import pallas as pl
from jax.experimental.pallas import tpu as pltpu

H = W = 512
C = 96
E = 384
NQ = 4
NG = C // 8
R = 16
RING = 4
LEAD = 3
EPS = 1e-5
_A = float(np.sqrt(2.0 / np.pi))
_S = (_A * 0.044715) ** (1.0 / 3.0)
_AP = _A / _S
f32, bf16 = jnp.float32, jnp.bfloat16

_FIRST = ("L0 L1 H0 L2 L3 E0 G4 H1 G12 I0 E1 H2 g18 E2 I1 A1 G21 D3 I2 D4 D5 D6 M C0 H7 I7 C1 E7 C2 C3 D8 "
          "C4 C5 D9 C6 C7 D10 C8 C9 O0 D11 C10 C11 O1 O2 O3 O4 O5")
_MID = ("L1 J0 G1 G2 J2 J1 L0 G4 J3 G5 J4 G6 L2 J5 G7 J6 G8 J7 G9 J8 G10 L3 J9 G11 J10 G12 J11 J12 G13 J13 "
        "G14 J14 G15 J15 G16 J16 G17 J19 G18 J18 G20 J17 J20 J21 A3 G22 J22 D4 J23 D5 D6 C0 M C1 D7 C2 C3 "
        "D8 C4 C5 D9 C6 C7 D10 C8 C9 D11 C10 C11 O0 O1 O2 O3 O4 O5")
_LAST = ("L1 L0 G0 G4 L2 x16 E0 L3 H0 g4 G6 I0 G8 E1 I1 E2 g11 H1 H2 I2 G20 D3 D4 D5 G22 E6 C0 H6 D7 M C1 "
         "C2 C3 A11 C4 C5 D8 I6 C6 C7 D9 D10 C8 C9 C10 D11 C11 O0 O1 O2 O3 O4 O5")

_XC, _CV, _ST, _DW, _TOK, _XN, _WT = 0, 4, 5, 6, 9, 10, 11
_NSLOT = 12


def _ls(q):
    return slice(128 * q, 128 * q + 128)


def _rs(g):
    return slice(8 * g, 8 * g + 8)


def _wslot(i):
    return _rs(i // 4), _ls(i % 4)


def _kernel(x_hbm, dw_ref, w1_ref, b1_ref, w2t_ref, b2_ref, g_ref, o_hbm,
            xin, xpre, obuf, vs, wts, acc_a, acc_b, b2b, zs, isem, osem, psem):
    nch, hr = H // R, R // 2

    def in_copy(j, slot, n=R):
        return pltpu.make_async_copy(x_hbm.at[pl.ds(j * R + LEAD, n)], xin.at[slot, pl.ds(0, n)], isem.at[slot])

    def out_copy(j, slot, p):
        return pltpu.make_async_copy(obuf.at[slot, pl.ds(p * hr, hr)],
                                     o_hbm.at[pl.ds(j * R + p * hr, hr)], osem.at[slot, p])

    pre = pltpu.make_async_copy(x_hbm.at[pl.ds(0, LEAD)], xpre, psem)
    pre.start()
    in_copy(0, 0).start()
    zs[0] = 0
    zs[1] = 0
    zs[2] = 0

    def bcast(row):
        r = jnp.concatenate([row, jnp.zeros((1, 128 - C), f32)], axis=1)
        return jnp.broadcast_to(r, (128, 128)).T[:C]

    vs[_XC + RING - 1] = jnp.zeros((C, W), f32)
    for t in range(9):
        vs[_DW + t // 4, :, _ls(t % 4)] = bcast(dw_ref[t // 3].astype(f32)[t % 3:t % 3 + 1])
    gb = bcast(g_ref[...].astype(f32).reshape(1, C))
    b2b[...] = gb * bcast(b2_ref[...].astype(f32).reshape(1, C))
    w1 = w1_ref[...].astype(f32)
    b1 = b1_ref[...].astype(f32).reshape(1, E) * _S
    b1h = b1.astype(bf16).astype(f32)
    cs = -jnp.sum(w1, axis=0, keepdims=True)
    csh = cs.astype(bf16).astype(f32)
    w1e = jnp.concatenate([w1, b1h, b1 - b1h, csh, cs - csh, jnp.zeros((128 - C - 4, E), f32)], axis=0).T
    for k in range(3):
        for c in range(8):
            v = pltpu.bitcast(w1e[128 * k + 16 * (7 - c):128 * k + 16 * (8 - c)].astype(bf16), f32)
            wts[(0,) + _wslot(8 * k + c)] = v
            vs[(_WT,) + _wslot(8 * k + c)] = v
    w2 = w2t_ref[...].astype(f32) * (jnp.concatenate([gb] * 3, axis=1) * (0.5 / _S))
    for k in range(3):
        for g in range(6):
            v = pltpu.bitcast(w2[16 * g:16 * g + 16, _ls(k)].astype(bf16), f32)
            wts[(0,) + _wslot(24 + 6 * k + g)] = v
            vs[(_WT,) + _wslot(24 + 6 * k + g)] = v

    lane = lax.broadcasted_iota(jnp.int32, (8, 128), 1)
    lane0, lane127 = lane == 0, lane == 127

    def load_rhs(za):
        return jnp.concatenate([vs[za + _XN], vs[za + _ST, 16:24, :], jnp.zeros((128 - C - 8, W), f32)], axis=0)

    class Conv:
        def __init__(s, src, n, za, zc):
            s.src, s.n, s.za, s.zc = src, n, za, zc
            s.st, s.s1, s.s2, s.done, s.stats = {}, [None] * NQ, [None] * NQ, 0, None

        def unpack(s, g):
            for q in range(NQ):
                vs[s.za + _XC + s.n % RING, _rs(g), _ls(q)] = s.src[_rs(g), _ls(q)].astype(f32)

        def taps(s, g, js, qs):
            def ldx(i, q):
                return vs[s.za + _XC + (s.n - 2 + i) % RING, _rs(g), _ls(q)]

            def ldw(j):
                return [vs[s.za + _DW + (3 * i + j) // 4, _rs(g), _ls((3 * i + j) % 4)] for i in range(3)]

            def fin(j, a):
                return pltpu.roll(a, 1, 1) if j == 0 else pltpu.roll(a, 127, 1) if j == 2 else a

            full = len(qs) == NQ
            cur = [list(t) if t else [None] * NQ for t in s.st.get(g, (None,) * 3)]
            if full and len(js) == 3:
                x = [[ldx(i, q) for q in qs] for i in range(3)]
                a = {}
                for j in js:
                    w = ldw(j)
                    a[j] = [x[0][q] * w[0] + x[1][q] * w[1] + x[2][q] * w[2] for q in qs]
                for j in js:
                    cur[j] = [fin(j, t) for t in a[j]]
            elif full:
                j = js[0]
                w = ldw(j)
                x = [[ldx(i, q) for q in qs] for i in range(3)]
                a = [x[0][q] * w[0] + x[1][q] * w[1] + x[2][q] * w[2] for q in qs]
                cur[j] = [fin(j, t) for t in a]
            else:
                j = js[0]
                w = ldw(j)
                for q in qs:
                    x = [ldx(i, q) for i in range(3)]
                    cur[j][q] = fin(j, x[0] * w[0] + x[1] * w[1] + x[2] * w[2])
            s.st[g] = cur

        def combine(s, g):
            left, mid, right = s.st.pop(g)
            for q in range(NQ):
                lo = jnp.where(lane0, left[q - 1] if q > 0 else 0.0, left[q])
                hi = jnp.where(lane127, right[q + 1] if q < NQ - 1 else 0.0, right[q])
                o = (lo + hi) + mid[q]
                s.s1[q] = o if s.s1[q] is None else s.s1[q] + o
                s.s2[q] = o * o if s.s2[q] is None else s.s2[q] + o * o
                vs[s.za + _CV, _rs(g), _ls(q)] = o
            s.done += 1
            if s.done == NG:
                for q in range(NQ):
                    vs[s.za + _ST, 0:8, _ls(q)] = s.s1[q]
                    vs[s.za + _ST, 8:16, _ls(q)] = s.s2[q]

        def _stats(s):
            sub = lax.broadcasted_iota(jnp.int32, (8, 128), 0)
            m4, m2 = sub < 4, (sub & 2) == 0

            def red(off):
                x = [vs[s.za + _ST, off:off + 8, _ls(q)] for q in range(NQ)]
                ab = jnp.where(m4, x[0], x[1]) + pltpu.roll(jnp.where(m4, x[1], x[0]), 4, 0)
                cd = jnp.where(m4, x[2], x[3]) + pltpu.roll(jnp.where(m4, x[3], x[2]), 4, 0)
                t = jnp.where(m2, ab + pltpu.roll(ab, 6, 0), cd + pltpu.roll(cd, 2, 0))
                return (t + pltpu.roll(t, 7, 0)) * (1.0 / C)

            m = red(0)
            r = lax.rsqrt(jnp.maximum(red(8) - m * m, 0.0) + EPS) * _S
            s.stats = (r, m * r)

        def norm(s, q):
            if s.stats is None:
                s._stats()
            k = (0, 4, 2, 6)[q]
            r, mr = (jnp.broadcast_to(t[k:k + 1, :], (8, 128)) for t in s.stats)
            for g in range(NG):
                vs[s.za + _XN, _rs(g), _ls(q)] = vs[s.za + _CV, _rs(g), _ls(q)] * r
            sub = lax.broadcasted_iota(jnp.int32, (8, 128), 0)
            vs[s.za + _ST, 16:24, _ls(q)] = jnp.where(sub < 2, 1.0, mr)

    def row(prog, cv, slot, dst, z, rhs, is_last):
        za, zb, zc = z
        steps = [(t[0], int(t[1:]) if len(t) > 1 else 0) for t in prog.split()]
        paced = {i for op, i in steps if op == 'x'}
        wl, st, acc, tok = {}, {'h': None, 'k': 0, 'rhs': rhs, 'u': 0}, [None] * NQ, {}

        def wload(i):
            if i not in wl:
                v = vs[(zc + _WT,) + _wslot(i)] if i - 24 in paced else wts[(0,) + _wslot(i)]
                wl[i] = pltpu.bitcast(v, bf16)
            return wl[i]

        def need(k):
            if st['h'] is None:
                y = jnp.dot(jnp.concatenate([wload(c) for c in range(24)], axis=0), rhs,
                            preferred_element_type=f32)
                st['h'] = [[[] for _ in range(NQ)] for _ in range(3)]
                for c in range(24):
                    for q in range(NQ):
                        yy = y[16 * c:16 * c + 16, _ls(q)]
                        h = yy * (jnp.tanh(yy * (yy * yy + _AP)) + 1.0)
                        st['h'][c // 8][q].append(h)
                        if q == 0:
                            tok['G', c] = tok['g', c] = h[0:8]
            while st['k'] <= k:
                kk = st['k']
                st['k'] += 1
                wk = jnp.concatenate([wload(24 + 6 * kk + g) for g in range(6)], axis=0)
                for q in range(NQ):
                    r = jnp.dot(wk, jnp.concatenate(st['h'][kk][q][::-1], axis=0), preferred_element_type=f32)
                    if kk == 0:
                        acc_a[za, :, _ls(q)] = r
                        if q == 0:
                            for g in range(NG):
                                tok['A', g] = r[_rs(g)]
                    elif kk == 1:
                        acc_b[za, :, _ls(q)] = r
                    else:
                        acc[q] = (r + acc_a[zb, :, _ls(q)]) + acc_b[zb, :, _ls(q)]

        for op, i in steps:
            if op in 'DEHIJ':
                g = i // 6 if op == 'J' else i
                while st['u'] <= g:
                    cv.unpack(st['u'])
                    st['u'] += 1
                if op == 'D':
                    cv.taps(g, (0, 2, 1), range(NQ))
                elif op == 'J':
                    cv.taps(g, ((0, 2, 1)[i % 3],), (0, 1) if i % 6 < 3 else (2, 3))
                else:
                    cv.taps(g, ({'E': 0, 'I': 1, 'H': 2}[op],), range(NQ))
            elif op == 'C':
                cv.combine(i)
            elif op == 'L':
                cv.norm(i)
            elif op in 'GAg':
                need(0 if op == 'A' else -1)
                vs[zc + _TOK, 0:8, 0:128] = tok[op, i]
            elif op == 'x':
                wload(24 + i)
            elif op == 'M':
                if not is_last:
                    st['rhs'] = load_rhs(za)
            elif op == 'O':
                need(2)
                for g in (2 * i, 2 * i + 1):
                    bb = b2b[_rs(g), :]
                    fin = [acc[q][_rs(g)] + (vs[za + _XC + slot, _rs(g), _ls(q)] + bb) for q in range(NQ)]
                    for h in range(2):
                        dst[_rs(g), 256 * h:256 * h + 256] = jnp.concatenate(fin[2 * h:2 * h + 2], axis=1).astype(bf16)
        return st['rhs']

    pre.wait()
    for n in range(LEAD):
        cv = Conv(xpre.at[n], n, zs[0], zs[2])
        for g in range(NG):
            cv.unpack(g)
        if n >= 1:
            for g in range(NG):
                cv.taps(g, (0, 2, 1), range(NQ))
                cv.combine(g)
        if n == 1:
            for q in range(NQ):
                cv.norm(q)

    def body(j, carry):
        slot = j % 2

        @pl.when(j + 1 < nch - 1)
        def _():
            in_copy(j + 1, 1 - slot).start()

        @pl.when(j + 1 == nch - 1)
        def _():
            in_copy(j + 1, 1 - slot, R - LEAD).start()
            xin[1 - slot, R - LEAD:R] = jnp.zeros((LEAD, C, W), bf16)

        @pl.when(j < nch - 1)
        def _():
            in_copy(j, slot).wait()

        @pl.when(j == nch - 1)
        def _():
            in_copy(j, slot, R - LEAD).wait()

        @pl.when(j >= 2)
        def _():
            out_copy(j - 2, slot, 0).wait()
            out_copy(j - 2, slot, 1).wait()

        z = (zs[0], zs[1], zs[2])
        rhs = load_rhs(z[0])
        for r in range(R):
            prog = _FIRST if r == 0 else _LAST if r == R - 1 else _MID
            rhs = row(prog, Conv(xin.at[slot, r], r + LEAD, z[0], z[2]), r % RING, obuf.at[slot, r], z, rhs,
                      r == R - 1)
            if (r + 1) % hr == 0:
                out_copy(j, slot, r // hr).start()
        return carry

    lax.fori_loop(0, nch, body, 0)
    for j in (nch - 2, nch - 1):
        out_copy(j, j % 2, 0).wait()
        out_copy(j, j % 2, 1).wait()


@jax.jit
def pallas_standalone__modern_conv_block_convnext__vision_kernel(x, dw, w1, b1, w2, b2, gamma):
    xt = jnp.transpose(x, (0, 1, 3, 2)).reshape(H, C, W)
    vm = pl.BlockSpec(memory_space=pltpu.VMEM)
    hbm = pl.BlockSpec(memory_space=pl.ANY)
    one = pltpu.VMEM((1, C, W), f32)
    out = pl.pallas_call(
        _kernel,
        in_specs=[hbm, vm, vm, vm, vm, vm, vm],
        out_specs=hbm,
        out_shape=jax.ShapeDtypeStruct((H, C, W), bf16),
        scratch_shapes=[
            pltpu.VMEM((2, R, C, W), bf16), pltpu.VMEM((LEAD, C, W), bf16), pltpu.VMEM((2, R, C, W), bf16),
            pltpu.VMEM((_NSLOT, C, W), f32), one, one, one, pltpu.VMEM((C, 128), f32),
            pltpu.SMEM((4,), jnp.int32),
            pltpu.SemaphoreType.DMA((2,)), pltpu.SemaphoreType.DMA((2, 2)), pltpu.SemaphoreType.DMA(()),
        ],
        compiler_params=pltpu.CompilerParams(
            vmem_limit_bytes=64 * 1024 * 1024, flags={"XLA_TPU_FORCE_LP_LLO_SCHEDULER": True}),
    )(xt, dw, w1, b1, w2.T, b2, gamma)
    return jnp.transpose(out.reshape(1, H, C, W), (0, 1, 3, 2))
```
